```python
import os as _os
_os.environ.setdefault("JAX_PLATFORMS", "cpu")
import jax
import jax.numpy as jnp

def _softmax(x, axis=-1):
    return jax.nn.softmax(x, axis=axis)
def _gelu(x):
    return jax.nn.gelu(x, approximate=True)
def _silu(x):
    return jax.nn.silu(x)
def _sigmoid(x):
    return jax.nn.sigmoid(x)
def _layernorm(x, axis=-1, eps=1e-5):
    m = jnp.mean(x, axis=axis, keepdims=True)
    v = jnp.var(x, axis=axis, keepdims=True)
    return (x - m) / jnp.sqrt(v + eps)
def _scatter_add(tgt, idx, src, axis=0):
    return tgt.at[idx].add(src)
def _segment_sum(src, seg, n):
    return jax.ops.segment_sum(src, seg, n)
class _Rng:
    def __init__(self, key):
        self._k = key
    def _next(self):
        self._k, sub = jax.random.split(self._k)
        return sub
    def normal(self, shape):
        return jax.random.normal(self._next(), shape, dtype=jnp.bfloat16)
    def randint(self, lo, hi, shape):
        return jax.random.randint(self._next(), shape, lo, hi, dtype=jnp.int32)
    def uniform(self, shape, lo=0.0, hi=1.0):
        return jax.random.uniform(self._next(), shape, jnp.bfloat16, lo, hi)
    def permutation(self, n):
        return jax.random.permutation(self._next(), n)


kernel_name = 'standalone__gqa_softmax__near_ridge'

def setup_inputs():
    _rng = _Rng(jax.random.key(int.from_bytes(__import__("os").urandom(4), "little")))
    _w = (lambda a: (lambda t: t.astype(jnp.bfloat16) if jnp.issubdtype(t.dtype, jnp.floating) else t)(jnp.asarray(a)))
    B, Hq, Hkv, Sq, Sk, D = 16, 32, 32, 368, 512, 192
    return {
        "q": _w((lambda *s: _rng.normal(s) * 0.4)(B, Hq, Sq, D)),
        "k": _w((lambda *s: _rng.normal(s) * 0.4)(B, Hkv, Sk, D)),
        "v": _w((lambda *s: _rng.normal(s) * 0.05)(B, Hkv, Sk, D)),
    }

def reference(q, k, v):
    B, Hq, Sq, D = q.shape
    Hkv = k.shape[1]
    rep = Hq // Hkv
    k = jnp.repeat(k, rep, axis=1)
    v = jnp.repeat(v, rep, axis=1)
    scale = D ** -0.5
    scores = jnp.einsum("bhqd,bhkd->bhqk", q, k) * scale
    p = _softmax(scores, axis=-1)
    return jnp.einsum("bhqk,bhkd->bhqd", p, v)
```

```python
import math

import jax
import jax.numpy as jnp
from jax import lax
import jax.experimental.pallas as pl
import jax.experimental.pallas.tpu as pltpu


@jax.jit
def pallas_standalone__gqa_softmax__near_ridge_kernel(
    q: jax.Array,
    k: jax.Array,
    v: jax.Array,
):
    B, Hq, Sq, D = q.shape
    _, Hkv, Sk, _ = k.shape
    assert Hq == Hkv
    n = B * Hq
    hb = 8
    c = (D ** -0.5) * math.log2(math.e)

    def kernel_function(q_ref, k_ref, v_ref, o_ref):
        for h in range(hb):
            s = lax.dot_general(q_ref[h], k_ref[h], (((0,), (0,)), ((), ())),
                                preferred_element_type=jnp.float32)
            m = jnp.max(s, axis=1, keepdims=True)
            p = jnp.exp2((s - m) * c).astype(jnp.bfloat16)
            v1 = jnp.concatenate([v_ref[h], jnp.ones((16, Sk), jnp.bfloat16)], axis=0)
            ot = lax.dot_general(v1, p, (((1,), (1,)), ((), ())),
                                 preferred_element_type=jnp.float32)
            o_ref[h] = (ot[:D] * (1.0 / ot[D:D + 1])).astype(o_ref.dtype)

    qt = jnp.swapaxes(q, 2, 3).reshape(n, D, Sq)
    kt = jnp.swapaxes(k, 2, 3).reshape(n, D, Sk)
    vt = jnp.swapaxes(v, 2, 3).reshape(n, D, Sk)
    im = lambda i: (i, 0, 0)
    ot = pl.pallas_call(
        kernel_function,
        grid=(n // hb,),
        in_specs=[pl.BlockSpec((hb, D, Sq), im), pl.BlockSpec((hb, D, Sk), im),
                  pl.BlockSpec((hb, D, Sk), im)],
        out_specs=pl.BlockSpec((hb, D, Sq), im),
        out_shape=jax.ShapeDtypeStruct((n, D, Sq), q.dtype),
        compiler_params=pltpu.CompilerParams(
            dimension_semantics=("arbitrary",), vmem_limit_bytes=100 * 1024 * 1024),
    )(qt, kt, vt)
    return jnp.swapaxes(ot.reshape(B, Hq, D, Sq), 2, 3)
```

```python
import math

import jax
import jax.numpy as jnp
from jax import lax
import jax.experimental.pallas as pl
import jax.experimental.pallas.tpu as pltpu

_QUAD = 4
_BIG = 16
_RAMP = 13
_SLOTS = 8
_WRITE_FROM = 404
_STREAMS = 8
_WRITE_ROWS = 48
_ROWS = 16
_LANES = 128

_NT = (((1,), (1,)), ((), ()))


def _after(x, marks, never):
    if not marks:
        return x
    parts = []
    for b in range(x.shape[0] // _ROWS):
        blk = x[_ROWS * b:_ROWS * (b + 1)]
        if b in marks:
            bits = pltpu.bitcast(blk[:, :_LANES], jnp.int32)
            for mark in marks[b]:
                bits = jnp.where(never, mark, bits)
            blk = jnp.concatenate(
                [pltpu.bitcast(bits, x.dtype), blk[:, _LANES:]], axis=1)
        parts.append(blk)
    return jnp.concatenate(parts, axis=0)


def _mark(col):
    half = _ROWS // 2
    both = jnp.maximum(col[:half], col[half:])
    return pltpu.bitcast(jnp.broadcast_to(both, (half, _LANES)), jnp.int32)


@jax.jit
def pallas_standalone__gqa_softmax__near_ridge_kernel(
    q: jax.Array,
    k: jax.Array,
    v: jax.Array,
):
    B, Hq, Sq, D = q.shape
    _, Hkv, Sk, _ = k.shape
    assert Hq == Hkv, "one K/V head per query head at these shapes"
    n = B * Hq
    dtype = q.dtype
    log2_scale = D ** -0.5 * math.log2(math.e)

    t_main = _QUAD * _RAMP
    n_main = (n - t_main) // _BIG
    t_last = t_main + n_main * _BIG
    ring = _SLOTS * _BIG
    shift = -t_main % _BIG
    ahead = _SLOTS - 1
    pv_rows, qk_rows = D // _ROWS, Sq // _ROWS
    q_tiles = pl.cdiv(Sq, _LANES)

    def kernel_function(q_hbm, k_hbm, v_hbm, o_hbm, qo, k_ring, v_ring,
                        s_carry, p_carry, read_sems, write_sem):
        def reads(step, t0, u, first=False, last=False):
            sem = read_sems.at[step % _SLOTS]
            r0 = (t0 + shift) % ring
            skip = 2 if first else 0
            nv = u - skip + (2 if last else 0)
            quads = pl.ds(t0 // _QUAD, u // _QUAD)
            copies = [
                pltpu.make_async_copy(q_hbm.at[quads], qo.at[quads], sem),
                pltpu.make_async_copy(
                    k_hbm.at[pl.ds(t0, u)], k_ring.at[pl.ds(r0, u)], sem),
            ] if u else []
            copies.append(pltpu.make_async_copy(
                v_hbm.at[pl.ds(t0 - 2 + skip, nv)],
                v_ring.at[pl.ds(r0 + skip, nv)], sem))
            return copies

        def ramp_reads(step, first=False):
            return reads(step, step * _QUAD, _QUAD, first=first)

        def main_reads(step):
            return reads(step, t_main + (step - _RAMP) * _BIG, _BIG)

        def last_reads():
            return reads(_RAMP + n_main, t_last, n - t_last, last=True)

        def start(copies):
            for copy in copies:
                copy.start()

        def wait(copies):
            for copy in copies:
                copy.wait()

        def write_quads(g0, count):
            for j in range(_QUAD):
                for r in range(0, D, _WRITE_ROWS):
                    idx = (pl.ds(g0, count), j, pl.ds(r, _WRITE_ROWS))
                    pltpu.make_async_copy(
                        qo.at[idx], o_hbm.at[idx], write_sem).start()

        def write_groups(lo, hi):
            def body(w, carry):
                write_quads(w * _STREAMS, _STREAMS)
                return carry
            lax.fori_loop(lo, hi, body, 0)

        def compute(t0, u, never, first=False, last=False):
            r0 = (t0 + shift) % ring
            g0 = t0 // _QUAD
            s_prev = None if first else s_carry[...]
            p_prev = None if first else p_carry[...]
            for t in range(u + (2 if last else 0)):
                marks, p_new = {}, None
                if s_prev is not None:
                    chunks = []
                    for j in range(qk_rows):
                        s = s_prev[_ROWS * j:_ROWS * (j + 1)]
                        m = jnp.max(s, axis=1, keepdims=True)
                        e = jnp.exp2((s - m) * log2_scale)
                        l = jnp.sum(e, axis=1, keepdims=True)
                        r = pltpu.reciprocal(l, approx=True)
                        r = r * (2.0 - l * r)
                        chunks.append((e * r).astype(dtype))
                        if p_prev is not None and t < u:
                            slot = 30 + 11 * j // 5
                            marks.setdefault(slot - 16, []).append(_mark(m))
                            marks.setdefault(slot, []).append(_mark(l))
                    p_new = jnp.concatenate(chunks, axis=0)

                def marks_in(lo, count):
                    return {b - lo: x for b, x in marks.items()
                            if lo <= b < lo + count}

                if t < u:
                    q_t = qo[g0 + t // _QUAD, t % _QUAD].T
                if p_prev is not None:
                    v_t = v_ring[r0 + t]
                    o_t = [
                        lax.dot_general(
                            _after(v_t, marks_in(pv_rows * j, pv_rows), never),
                            p_prev[_LANES * j:_LANES * (j + 1)], _NT,
                            preferred_element_type=jnp.float32).astype(dtype)
                        for j in range(q_tiles)]
                    qo[g0 + (t - 2) // _QUAD, (t - 2) % _QUAD] = (
                        jnp.concatenate(o_t, axis=1))
                s_prev = None
                if t < u:
                    k_t = k_ring[r0 + t]
                    s_prev = jnp.concatenate([
                        jnp.dot(
                            _after(q_t, marks_in(
                                pv_rows * q_tiles + qk_rows * j, qk_rows), never),
                            k_t[:, Sk // 2 * j:Sk // 2 * (j + 1)],
                            preferred_element_type=jnp.float32)
                        for j in range(2)], axis=1)
                p_prev = p_new
            if not last:
                s_carry[...] = s_prev
                p_carry[...] = p_prev

        start(ramp_reads(0, first=True))
        for step in range(1, ahead + 1):
            start(ramp_reads(step))
        wait(ramp_reads(0, first=True))

        def ramp_step(step, carry):
            @pl.when(step == 0)
            def _():
                compute(0, _QUAD, step < 0, first=True)

            @pl.when(step > 0)
            def _():
                @pl.when(step + ahead < _RAMP)
                def _():
                    start(ramp_reads(step + ahead))

                @pl.when(step + ahead >= _RAMP)
                def _():
                    start(main_reads(step + ahead))

                wait(ramp_reads(step))
                compute(step * _QUAD, _QUAD, step < 0)
            return carry

        lax.fori_loop(0, _RAMP, ramp_step, 0)

        group = _QUAD * _STREAMS
        i_write = (_WRITE_FROM - t_main) // _BIG

        def main_step(i, written):
            step, t0 = _RAMP + i, t_main + i * _BIG

            @pl.when(i + ahead < n_main)
            def _():
                start(main_reads(step + ahead))

            @pl.when(i + ahead == n_main)
            def _():
                start(last_reads())

            target = jnp.minimum(3 + (i - i_write) * 19 // 8, (t0 - 2) // group)
            target = jnp.where(i >= i_write, target, 0)
            write_groups(written, target)
            wait(main_reads(step))
            compute(t0, _BIG, i < 0)
            return target

        written = lax.fori_loop(0, n_main, main_step, jnp.int32(0))

        groups_done = (t_last - 2) // group
        quads_done = (t_last - 2) // _QUAD
        write_groups(written, groups_done)
        if quads_done > groups_done * _STREAMS:
            write_quads(groups_done * _STREAMS,
                        quads_done - groups_done * _STREAMS)
        wait(last_reads())
        compute(t_last, n - t_last, written < 0, last=True)
        write_quads(quads_done, n // _QUAD - quads_done)
        pltpu.make_async_copy(qo, o_hbm, write_sem).wait()

    quad_shape = (n // _QUAD, _QUAD, D, Sq)
    o_t = pl.pallas_call(
        kernel_function,
        in_specs=[pl.BlockSpec(memory_space=pl.ANY)] * 3,
        out_specs=pl.BlockSpec(memory_space=pl.ANY),
        out_shape=jax.ShapeDtypeStruct(quad_shape, dtype),
        scratch_shapes=[
            pltpu.VMEM(quad_shape, dtype),
            pltpu.VMEM((ring, D, Sk), dtype),
            pltpu.VMEM((ring, D, Sk), dtype),
            pltpu.VMEM((Sq, Sk), jnp.float32),
            pltpu.VMEM((Sq, Sk), dtype),
            pltpu.SemaphoreType.DMA((_SLOTS,)),
            pltpu.SemaphoreType.DMA(()),
        ],
        compiler_params=pltpu.CompilerParams(
            vmem_limit_bytes=127 * 1024 * 1024, disable_bounds_checks=True),
    )(
        jnp.swapaxes(q, 2, 3).reshape(quad_shape),
        jnp.swapaxes(k, 2, 3).reshape(n, D, Sk),
        jnp.swapaxes(v, 2, 3).reshape(n, D, Sk),
    )
    return jnp.swapaxes(o_t.reshape(B, Hq, D, Sq), 2, 3)
```

```python
import math

import jax
import jax.numpy as jnp
from jax import lax
import jax.experimental.pallas as pl
import jax.experimental.pallas.tpu as pltpu

_LEAD = 2
_QUAD = 4
_BIG = 16
_RAMP = 12
_SLOTS = 8
_WRITE_FROM = 400
_STREAMS = 8
_WRITE_ROWS = 48
_TAIL = (12, 4)
_CHUNK = 16
_LANES = 128


@jax.jit
def pallas_standalone__gqa_softmax__near_ridge_kernel(
    q: jax.Array,
    k: jax.Array,
    v: jax.Array,
):
    B, Hq, Sq, D = q.shape
    _, Hkv, Sk, _ = k.shape
    assert Hq == Hkv, "one K/V head per query head at these shapes"
    n = B * Hq
    dtype = q.dtype
    log2_scale = D ** -0.5 * math.log2(math.e)

    h_main = _QUAD * _RAMP
    h_last = n - _BIG
    n_main = (h_last - h_main) // _BIG
    ring = _SLOTS * _BIG
    ahead = _SLOTS - 1
    assert h_main % _BIG == 0 and n % _BIG == 0 and sum(_TAIL) == _BIG
    assert ahead <= _RAMP and ahead <= n_main and h_main >= 2 * _BIG

    def scores(q_t, k_t):
        q_h = q_t.T
        return jnp.concatenate([
            jnp.dot(q_h, k_t[:, c:c + Sk // 2],
                    preferred_element_type=jnp.float32)
            for c in (0, Sk // 2)], axis=1)

    def softmax(s):
        chunks = []
        for r in range(0, Sq, _CHUNK):
            x = s[r:r + _CHUNK]
            m = jnp.max(x, axis=1, keepdims=True)
            e = jnp.exp2((x - m) * log2_scale)
            l = jnp.sum(e, axis=1, keepdims=True)
            inv = pltpu.reciprocal(l, approx=True)
            inv = inv * (2.0 - l * inv)
            chunks.append((e * inv).astype(dtype))
        return jnp.concatenate(chunks, axis=0)

    def weighted_values(v_t, p):
        return jnp.concatenate([
            lax.dot_general(v_t, p[r:r + _LANES], (((1,), (1,)), ((), ())),
                            preferred_element_type=jnp.float32).astype(dtype)
            for r in range(0, Sq, _LANES)], axis=1)

    def kernel_function(q_hbm, k_hbm, v_hbm, o_hbm, qo, k_ring, v_ring,
                        s_carry, p_carry, read_sems, write_sem):
        def reads(step, h0, u, last=False):
            sem = read_sems.at[step % _SLOTS]
            quads = pl.ds(h0 // _QUAD + 1, u // _QUAD - (1 if last else 0))
            nk = u - (_LEAD if last else 0)
            return [
                pltpu.make_async_copy(q_hbm.at[quads], qo.at[quads], sem),
                pltpu.make_async_copy(k_hbm.at[pl.ds(h0 + _LEAD, nk)],
                                      k_ring.at[pl.ds(h0 % ring, nk)], sem),
                pltpu.make_async_copy(v_hbm.at[pl.ds(h0, u)],
                                      v_ring.at[pl.ds(h0 % ring, u)], sem),
            ]

        def first_reads():
            sem = read_sems.at[_SLOTS - 1]
            return [
                pltpu.make_async_copy(q_hbm.at[0], qo.at[0], sem),
                pltpu.make_async_copy(k_hbm.at[pl.ds(0, _LEAD)],
                                      k_ring.at[pl.ds(ring - _LEAD, _LEAD)], sem),
            ]

        def ramp_reads(step):
            return reads(step, step * _QUAD, _QUAD)

        def main_reads(step):
            return reads(step, h_main + (step - _RAMP) * _BIG, _BIG)

        def last_reads():
            return reads(_RAMP + n_main, h_last, _BIG, last=True)

        def start(copies):
            for copy in copies:
                copy.start()

        def wait(copies):
            for copy in copies:
                copy.wait()

        def write_quads(g0, count):
            for j in range(_QUAD):
                for r in range(0, D, _WRITE_ROWS):
                    idx = (pl.ds(g0, count), j, pl.ds(r, _WRITE_ROWS))
                    pltpu.make_async_copy(
                        qo.at[idx], o_hbm.at[idx], write_sem).start()

        def write_groups(lo, hi):
            def body(w, carry):
                write_quads(w * _STREAMS, _STREAMS)
                return carry
            lax.fori_loop(lo, hi, body, 0)

        def compute(h0, u, last=False):
            r0, g0 = h0 % ring, h0 // _QUAD
            s, p = s_carry[...], p_carry[...]
            for i in range(u):
                more = not last or i + _LEAD < u
                p_next = softmax(s) if s is not None else None
                if more:
                    q_t = qo[g0 + (i + _LEAD) // _QUAD, (i + _LEAD) % _QUAD]
                qo[g0 + i // _QUAD, i % _QUAD] = weighted_values(
                    v_ring[r0 + i], p)
                s = scores(q_t, k_ring[r0 + i]) if more else None
                p = p_next
            if not last:
                s_carry[...] = s
                p_carry[...] = p

        start(first_reads())
        for step in range(ahead):
            start(ramp_reads(step))
        wait(first_reads())
        p_carry[...] = softmax(scores(qo[0, 0], k_ring[ring - 2]))
        s_carry[...] = scores(qo[0, 1], k_ring[ring - 1])

        def ramp_step(step, carry):
            @pl.when(step + ahead < _RAMP)
            def _():
                start(ramp_reads(step + ahead))

            @pl.when(step + ahead >= _RAMP)
            def _():
                start(main_reads(step + ahead))

            wait(ramp_reads(step))
            compute(step * _QUAD, _QUAD)
            return carry

        lax.fori_loop(0, _RAMP, ramp_step, 0)

        group = _QUAD * _STREAMS
        i_write = (_WRITE_FROM - h_main) // _BIG

        def main_step(i, written):
            step, h0 = _RAMP + i, h_main + i * _BIG

            @pl.when(i + ahead < n_main)
            def _():
                start(main_reads(step + ahead))

            @pl.when(i + ahead == n_main)
            def _():
                start(last_reads())

            target = jnp.minimum(3 + (i - i_write) * 19 // 8, h0 // group)
            target = jnp.where(i >= i_write, target, 0)
            write_groups(written, target)
            wait(main_reads(step))
            compute(h0, _BIG)
            return target

        written = lax.fori_loop(0, n_main, main_step, jnp.int32(0))

        write_groups(written, h_last // group)
        if h_last % group:
            write_quads(h_last // group * _STREAMS, h_last % group // _QUAD)
        wait(last_reads())
        h0 = h_last
        for u in _TAIL:
            compute(h0, u, last=h0 + u == n)
            write_quads(h0 // _QUAD, u // _QUAD)
            h0 += u
        pltpu.make_async_copy(qo, o_hbm, write_sem).wait()

    quad_shape = (n // _QUAD, _QUAD, D, Sq)
    o_t = pl.pallas_call(
        kernel_function,
        in_specs=[pl.BlockSpec(memory_space=pl.ANY)] * 3,
        out_specs=pl.BlockSpec(memory_space=pl.ANY),
        out_shape=jax.ShapeDtypeStruct(quad_shape, dtype),
        scratch_shapes=[
            pltpu.VMEM(quad_shape, dtype),
            pltpu.VMEM((ring, D, Sk), dtype),
            pltpu.VMEM((ring, D, Sk), dtype),
            pltpu.VMEM((Sq, Sk), jnp.float32),
            pltpu.VMEM((Sq, Sk), dtype),
            pltpu.SemaphoreType.DMA((_SLOTS,)),
            pltpu.SemaphoreType.DMA(()),
        ],
        compiler_params=pltpu.CompilerParams(
            vmem_limit_bytes=127 * 1024 * 1024, disable_bounds_checks=True),
    )(
        jnp.swapaxes(q, 2, 3).reshape(quad_shape),
        jnp.swapaxes(k, 2, 3).reshape(n, D, Sk),
        jnp.swapaxes(v, 2, 3).reshape(n, D, Sk),
    )
    return jnp.swapaxes(o_t.reshape(B, Hq, D, Sq), 2, 3)
```

```python
import math

import jax
import jax.numpy as jnp
from jax import lax
import jax.experimental.pallas as pl
import jax.experimental.pallas.tpu as pltpu

_LEAD = 2
_QUAD = 4
_BIG = 16
_RAMP = 12
_SLOTS = 8
_WRITE_FROM = 400
_STREAMS = 6
_WRITE_ROWS = 48
_TAIL = (12, 4)
_LANES = 128


@jax.jit
def pallas_standalone__gqa_softmax__near_ridge_kernel(
    q: jax.Array,
    k: jax.Array,
    v: jax.Array,
):
    B, Hq, Sq, D = q.shape
    _, Hkv, Sk, _ = k.shape
    assert Hq == Hkv, "one K/V head per query head at these shapes"
    n = B * Hq
    dtype = q.dtype
    log2_scale = D ** -0.5 * math.log2(math.e)

    h_main = _QUAD * _RAMP
    h_last = n - _BIG
    n_main = (h_last - h_main) // _BIG
    ring = _SLOTS * _BIG
    ahead = _SLOTS - 1
    assert h_main % _BIG == 0 and n % _BIG == 0 and sum(_TAIL) == _BIG
    assert ahead <= _RAMP and ahead <= n_main and h_main >= 2 * _BIG
    assert D % _WRITE_ROWS == 0

    def scores(q_t, k_t):
        q_h = q_t.T
        return jnp.concatenate([
            jnp.dot(q_h, k_t[:, c:c + Sk // 2],
                    preferred_element_type=jnp.float32)
            for c in (0, Sk // 2)], axis=1)

    def softmax(s):
        m = jnp.max(s, axis=1, keepdims=True)
        e = jnp.exp2((s - m) * log2_scale)
        l = jnp.sum(e, axis=1, keepdims=True)
        inv = pltpu.reciprocal(l, approx=True)
        inv = inv * (2.0 - l * inv)
        return (e * inv).astype(dtype)

    def weighted_values(v_t, p):
        return jnp.concatenate([
            lax.dot_general(v_t, p[r:r + _LANES], (((1,), (1,)), ((), ())),
                            preferred_element_type=jnp.float32).astype(dtype)
            for r in range(0, Sq, _LANES)], axis=1)

    def kernel_function(q_hbm, k_hbm, v_hbm, o_hbm, qo, k_ring, v_ring,
                        s_carry, p_carry, read_sems, write_sem):
        def reads(step, h0, u, last=False):
            sem = read_sems.at[step % _SLOTS]
            quads = pl.ds(h0 // _QUAD + 1, u // _QUAD - (1 if last else 0))
            nk = u - (_LEAD if last else 0)
            return [
                pltpu.make_async_copy(q_hbm.at[quads], qo.at[quads], sem),
                pltpu.make_async_copy(k_hbm.at[pl.ds(h0 + _LEAD, nk)],
                                      k_ring.at[pl.ds(h0 % ring, nk)], sem),
                pltpu.make_async_copy(v_hbm.at[pl.ds(h0, u)],
                                      v_ring.at[pl.ds(h0 % ring, u)], sem),
            ]

        def first_reads():
            sem = read_sems.at[_SLOTS - 1]
            return [
                pltpu.make_async_copy(q_hbm.at[0], qo.at[0], sem),
                pltpu.make_async_copy(k_hbm.at[pl.ds(0, _LEAD)],
                                      k_ring.at[pl.ds(ring - _LEAD, _LEAD)], sem),
            ]

        def ramp_reads(step):
            return reads(step, step * _QUAD, _QUAD)

        def main_reads(step):
            return reads(step, h_main + (step - _RAMP) * _BIG, _BIG)

        def last_reads():
            return reads(_RAMP + n_main, h_last, _BIG, last=True)

        def start(copies):
            for copy in copies:
                copy.start()

        def wait(copies):
            for copy in copies:
                copy.wait()

        def write_quads(g0, count):
            for j in range(_QUAD):
                for r in range(0, D, _WRITE_ROWS):
                    idx = (pl.ds(g0, count), j, pl.ds(r, _WRITE_ROWS))
                    pltpu.make_async_copy(
                        qo.at[idx], o_hbm.at[idx], write_sem).start()

        def write_groups(lo, hi):
            def body(w, carry):
                write_quads(w * _STREAMS, _STREAMS)
                return carry
            lax.fori_loop(lo, hi, body, 0)

        def compute(h0, u, last=False):
            r0, g0 = h0 % ring, h0 // _QUAD
            s, p = s_carry[...], p_carry[...]
            for i in range(u):
                more = not last or i + _LEAD < u
                p_next = softmax(s) if s is not None else None
                if more:
                    q_t = qo[g0 + (i + _LEAD) // _QUAD, (i + _LEAD) % _QUAD]
                qo[g0 + i // _QUAD, i % _QUAD] = weighted_values(
                    v_ring[r0 + i], p)
                s = scores(q_t, k_ring[r0 + i]) if more else None
                p = p_next
            if not last:
                s_carry[...] = s
                p_carry[...] = p

        start(first_reads())
        for step in range(ahead):
            start(ramp_reads(step))
        wait(first_reads())
        p_carry[...] = softmax(scores(qo[0, 0], k_ring[ring - 2]))
        s_carry[...] = scores(qo[0, 1], k_ring[ring - 1])

        def ramp_step(step, carry):
            @pl.when(step + ahead < _RAMP)
            def _():
                start(ramp_reads(step + ahead))

            @pl.when(step + ahead >= _RAMP)
            def _():
                start(main_reads(step + ahead))

            wait(ramp_reads(step))
            compute(step * _QUAD, _QUAD)
            return carry

        lax.fori_loop(0, _RAMP, ramp_step, 0)

        group = _QUAD * _STREAMS
        i_write = (_WRITE_FROM - h_main) // _BIG

        def main_step(i, written):
            step, h0 = _RAMP + i, h_main + i * _BIG

            @pl.when(i + ahead < n_main)
            def _():
                start(main_reads(step + ahead))

            @pl.when(i + ahead == n_main)
            def _():
                start(last_reads())

            target = jnp.minimum(4 + 3 * (i - i_write), h0 // group)
            target = jnp.where(i >= i_write, target, 0)
            write_groups(written, target)
            wait(main_reads(step))
            compute(h0, _BIG)
            return target

        written = lax.fori_loop(0, n_main, main_step, jnp.int32(0))

        write_groups(written, h_last // group)
        if h_last % group:
            write_quads(h_last // group * _STREAMS, h_last % group // _QUAD)
        wait(last_reads())
        h0 = h_last
        for u in _TAIL:
            compute(h0, u, last=h0 + u == n)
            write_quads(h0 // _QUAD, u // _QUAD)
            h0 += u
        pltpu.make_async_copy(qo, o_hbm, write_sem).wait()

    quad_shape = (n // _QUAD, _QUAD, D, Sq)
    o_t = pl.pallas_call(
        kernel_function,
        in_specs=[pl.BlockSpec(memory_space=pl.ANY)] * 3,
        out_specs=pl.BlockSpec(memory_space=pl.ANY),
        out_shape=jax.ShapeDtypeStruct(quad_shape, dtype),
        scratch_shapes=[
            pltpu.VMEM(quad_shape, dtype),
            pltpu.VMEM((ring, D, Sk), dtype),
            pltpu.VMEM((ring, D, Sk), dtype),
            pltpu.VMEM((Sq, Sk), jnp.float32),
            pltpu.VMEM((Sq, Sk), dtype),
            pltpu.SemaphoreType.DMA((_SLOTS,)),
            pltpu.SemaphoreType.DMA(()),
        ],
        compiler_params=pltpu.CompilerParams(
            vmem_limit_bytes=126 * 1024 * 1024, disable_bounds_checks=True),
    )(
        jnp.swapaxes(q, 2, 3).reshape(quad_shape),
        jnp.swapaxes(k, 2, 3).reshape(n, D, Sk),
        jnp.swapaxes(v, 2, 3).reshape(n, D, Sk),
    )
    return jnp.swapaxes(o_t.reshape(B, Hq, D, Sq), 2, 3)
```
